```python
import os as _os
_os.environ.setdefault('JAX_PLATFORMS', 'cpu')
import jax
import jax.numpy as jnp

def _softmax(x, axis=-1):
    return jax.nn.softmax(x, axis=axis)

def _gelu(x):
    return jax.nn.gelu(x, approximate=True)

def _silu(x):
    return jax.nn.silu(x)

def _sigmoid(x):
    return jax.nn.sigmoid(x)

def _layernorm(x, axis=-1, eps=1e-05):
    m = jnp.mean(x, axis=axis, keepdims=True)
    v = jnp.var(x, axis=axis, keepdims=True)
    return (x - m) / jnp.sqrt(v + eps)

def _scatter_add(tgt, idx, src, axis=0):
    return tgt.at[idx].add(src)

def _segment_sum(src, seg, n):
    return jax.ops.segment_sum(src, seg, n)

class _Rng:

    def __init__(self, key):
        self._k = key

    def _next(self):
        self._k, sub = jax.random.split(self._k)
        return sub

    def normal(self, shape):
        return jax.random.normal(self._next(), shape, dtype=jnp.bfloat16)

    def randint(self, lo, hi, shape):
        return jax.random.randint(self._next(), shape, lo, hi, dtype=jnp.int32)

    def uniform(self, shape, lo=0.0, hi=1.0):
        return jax.random.uniform(self._next(), shape, jnp.bfloat16, lo, hi)

    def permutation(self, n):
        return jax.random.permutation(self._next(), n)
kernel_name = 'adaLN_cond__sliding_local_dilated__dense_activation_silu__prompt'

def setup_inputs():
    _rng = _Rng(jax.random.key(int.from_bytes(__import__("os").urandom(4), "little")))
    _w = lambda a: (lambda t: t.astype(jnp.bfloat16) if jnp.issubdtype(t.dtype, jnp.floating) else t)(jnp.asarray(a))

    def _A_setup():
        B, S, D = (1, 2048, 512)
        return {'x': _w((lambda *s: _rng.normal(s) * 0.05)(B, S, D)), 'wqkv': _w((lambda *s: _rng.normal(s) * 0.05)(D, 3 * D)), 'wo': _w((lambda *s: _rng.normal(s) * 0.05)(D, D))}
    _A_in = _A_setup()

    def _B_setup():
        B, S, D, F = (1, 2048, 512, 1792)
        return {'x': _w((lambda *s: _rng.normal(s) * 0.05)(B, S, D)), 'w1': _w((lambda *s: _rng.normal(s) * 0.8)(D, F) * D ** (-0.5)), 'w2': _w((lambda *s: _rng.normal(s) * 0.8)(F, D) * F ** (-0.5))}
    _B_in = _B_setup()
    return {'A_x': _A_in['x'], 'A_wqkv': _A_in['wqkv'], 'A_wo': _A_in['wo'], 'B_x': _B_in['x'], 'B_w1': _B_in['w1'], 'B_w2': _B_in['w2'], 'c': _w((lambda *s: _rng.normal(s) * 0.05)(1, 512) * 8.0), 'w_mod': _w((lambda *s: _rng.normal(s) * 0.05)(512, 6 * 512) * 512 ** (-0.5) * 8.0)}

def reference(A_x, A_wqkv, A_wo, B_x, B_w1, B_w2, c, w_mod):

    def _A_ref(x, wqkv, wo):
        B, S, D = x.shape
        H = 32
        Dh = D // H
        W, dil = (8, 2)
        qkv = (lambda x, *d: x.transpose(*d))((x @ wqkv).reshape(B, S, 3, H, Dh), 2, 0, 3, 1, 4)
        q, k, v = (qkv[0], qkv[1], qkv[2])
        scale = Dh ** (-0.5)
        pos = jnp.arange(S)
        off = jnp.arange(W) * dil
        idx = pos[:, None] - off[None, :]
        mask = idx >= 0
        idx_c = jnp.where(mask, idx, 0).reshape(-1)
        kg = k[:, :, idx_c, :].reshape(B, H, S, W, Dh)
        vg = v[:, :, idx_c, :].reshape(B, H, S, W, Dh)
        logits = jnp.einsum('bhsd,bhswd->bhsw', q, kg) * scale
        logits = jnp.where(mask[None, None, :, :], logits, -1000000000.0)
        attn = _softmax(logits, axis=-1)
        o = jnp.einsum('bhsw,bhswd->bhsd', attn, vg)
        return (lambda x, *d: x.transpose(*d))(o, 0, 2, 1, 3).reshape(B, S, D) @ wo

    def _B_ref(x, w1, w2):
        h = jnp.einsum('bsd,df->bsf', x, w1)
        h = _silu(h)
        out = jnp.einsum('bsf,fd->bsd', h, w2)
        return out
    x = A_x
    mod = (_silu(c) @ w_mod).reshape(c.shape[0], 6, 1, -1)
    sa, ca, ga, sb, cb, gb = (mod[:, 0].copy(), mod[:, 1].copy(), mod[:, 2].copy(), mod[:, 3].copy(), mod[:, 4].copy(), mod[:, 5].copy())
    h = _layernorm(x, axis=-1) * (1 + ca) + sa
    x = x + ga * _A_ref(h, A_wqkv, A_wo)
    h = _layernorm(x, axis=-1) * (1 + cb) + sb
    x = x + gb * _B_ref(h, B_w1, B_w2)
    return x
```

```python
import jax
import jax.numpy as jnp
from jax import lax
import jax.experimental.pallas as pl
import jax.experimental.pallas.tpu as pltpu

S, D, F = 2048, 512, 1792
H, DH, W, DIL = 32, 16, 8, 2
T = 128
NT, FT = D // T, F // T
BM = 512
NB, HB, QB = S // BM, BM // 2, BM // 4
HALO = 16
SPARE = 16
LOG2E = 1.4426950408889634
f32, bf16, u32 = jnp.float32, jnp.bfloat16, jnp.uint32

ORDER = ("Q00:3,Q00b,Q01,Q02,Q10,Q11,Q12,Q20,Q21,Q22,O0,Q30,Q31,Q32,"
         "F0,O1,G0:26,F1,G0b,O2,G1:24,F2,O3,G1b,F3,G2,G3")
ARRIVALS = {"Q00b": 4, "Q01": 5, "Q02": 6, "Q11": 7, "Q30": 8}
LOAD = dict(Q=0.55, O=0.85, F=1.05, G=0.7, F0=1.8)
PEAK, BURST = 3.0, 3.5
MARGIN, SETTLE = 150, 250
NEAR, FAR = 220, 370
EAGER = 1.1

_LHS = (((1, 0, 1), (1, 1, 1)), ((1, 1, 1),), ((0, 0, 1),), ((0, 0, 1), (0, 1, 1)),
        ((0, 0, 1), (1, 1, 1)), ((0, 1, 1), (1, 1, -1)), ((1, 0, 1), (0, 0, -1)))
_RHS = (((0, 0, 1),), ((1, 0, 1), (0, 0, -1)), ((0, 1, 1), (1, 1, -1)), ((1, 1, 1),),
        ((0, 0, 1), (1, 1, 1)), ((1, 0, 1), (1, 1, 1)), ((0, 0, 1), (0, 1, 1)))
SHARE = ((0, 1), (2, 3), (4,), (5,), (6,))


def _tree(f, xs):
    while len(xs) > 1:
        xs = [f(a, b) for a, b in zip(xs[::2], xs[1::2])]
    return xs[0]


def _signed_sum(terms, get):
    acc = get(*terms[0][:2])
    for i, j, sign in terms[1:]:
        acc = acc + get(i, j) if sign > 0 else acc - get(i, j)
    return acc


def _operands(table, tile, out):
    x = [[tile(i, j) for j in range(2)] for i in range(2)]
    for o, terms in enumerate(table):
        out(o, _signed_sum(terms, lambda i, j: x[i][j]))


def _operands2(table, outer, tile, out):
    seen = {}

    def once(i, j):
        if (i, j) not in seen:
            seen[i, j] = tile(i, j)
        return seen[i, j]

    for o in outer:
        block = lambda i, j: _signed_sum(table[o], lambda a, c: once(2 * a + i, 2 * c + j))
        _operands(table, block, lambda p, v: out(7 * o + p, v))


def _combiner(keep):
    t = []

    def step(r, m):
        if r < 5:
            t.append(keep(m, (2, 1, 2, 1, 2)[r]))
        if r == 1:
            return 1, 0, t[0]() + m
        if r == 3:
            return 0, 1, t[2]() + m
        if r == 5:
            return 0, 0, (t[1]() - t[3]()) + (t[4]() + m)
        if r == 6:
            return 1, 1, (t[2]() - t[0]()) + (t[4]() + m)
    return step


def _rates(room, jobs):
    rate = {}
    while jobs:
        best = (-1.0,)
        for a in sorted({j[1] for j in jobs}):
            for z in sorted({j[2] for j in jobs}):
                space = sum(room[i] for i in range(a, z) if i not in rate)
                if space:
                    best = max(best, (sum(j[0] for j in jobs if a <= j[1] and j[2] <= z) / space, a, z))
        r, a, z = best
        rate.update({i: r for i in range(a, z) if i not in rate})
        jobs = [(w, z if a <= s < z else s, a if a < e <= z else e) for w, s, e in jobs if not (a <= s and e <= z)]
    return [rate.get(i, 0.0) for i in range(len(room))]


def _emit(stages, tasks, eager):
    index = {st[0]: i for i, st in enumerate(stages)}
    tasks = [[ops, index[a.rstrip("+")] + 1, index[z], gen, SETTLE * a.count("+"), dense]
             for dense, group in enumerate(tasks) for ops, a, z, gen in group]
    tasks.sort(key=lambda k: k[2])
    rates = _rates([cyc * (PEAK - load) for _, cyc, load, _ in stages], [tuple(k[:3]) for k in tasks])
    credit = quota = used = mix = 0.0
    for i, (_, cyc, load, gen) in enumerate(stages):
        while tasks and tasks[0][2] <= i:
            sum(tasks.pop(0)[3])
        t = 0
        for c in gen:
            t += c
            quota += c * EAGER
            used = max(used - c * BURST, 0.0)
            while eager and quota > 0:
                step = next(eager[0], None)
                if step is None:
                    eager.pop(0)
                else:
                    quota -= step[0]
                    used += step[1]
            quota = min(quota, 0.0)
            due = sum(k[0] for k in tasks if k[2] == i + 1)
            credit += c * max((PEAK - load) * rates[i], due / max(cyc - t - MARGIN, 16))
            while credit > 0 and used < 0.7 * c * BURST:
                ready = [k for k in tasks if k[1] < i or (k[1] == i and t > k[4])]
                if not ready:
                    break
                need, first = [0.0, 0.0], {}
                for dense in range(2):
                    total = 0
                    for k in ready:
                        if k[5] == dense:
                            first.setdefault(dense, k)
                            total += max(k[0], 1)
                            left = sum(st[1] for st in stages[i:k[2]]) - t - MARGIN
                            need[dense] = max(need[dense], total / max(left, 16))
                task = first[int(mix > 0)] if len(first) == 2 else ready[0]
                ops = next(task[3], None)
                if ops is None:
                    tasks.remove(task)
                else:
                    task[0] -= ops
                    credit -= ops
                    used += ops
                    mix += ops * (need[1] / sum(need) - task[5])
            credit = min(credit, 100.0)
    assert not tasks


def _scratch():
    buf = lambda *shape, dtype=f32: pltpu.VMEM(shape[:-2] + (shape[-2] + SPARE, shape[-1]), dtype)
    half = lambda *shape: buf(*shape, dtype=bf16)
    landing = dict(x=[half(BM, D)] * NB, wqkv=[half(D, D)] * 3, wmod=[half(D, D)] * 6,
                   wo=half(D, D), w1=half(D, F), w2=half(F, D), c=pltpu.VMEM((1, D), bf16))
    tied = dict(
        mod=[buf(NT, 8, T)] * 6, perm=[buf(NT * NT, T // 4, T, dtype=u32)] * 2,
        bq=[half(7, 2, 2 * T, T)] * 3, bo=half(7, 2, 2 * T, T), b1=half(7, FT // 2, 2 * T, T),
        b2=half(49, 1, 3 * T, T), b2r=half(7, 2, T, T),
        aq=[half(7, 2, HB, T)] * 2, ao=[half(7, 2, HB, T)] * 2, a1=[half(7, 2, HB, T)] * 2,
        a2=[half(49, 3, QB, T)] * 2, a2r=[half(7, 1, HB, T)] * 2,
        stats=[[[buf(BM, T)] * 2] * 2] * 2, logit=[buf(W, 8, T)] * 8, prob=[buf(W, 8, T)] * 8,
        att=[buf(NT, 32, T)] * 4)
    other = dict(
        sc=pltpu.VMEM((D, T), f32), wo32=buf(NT, H * (DH + 1), T), q=[buf(NT, BM, T)] * NB,
        k=pltpu.VMEM((NT, HALO + S, T), f32), v=pltpu.VMEM((NT, HALO + S, T), f32), x1=[buf(NT, BM, T)] * NB,
        hid=[[pltpu.VMEM((BM, T), f32)] * FT] * 2, tmp=[pltpu.VMEM((HB, T), f32)] * 48,
        out=pltpu.VMEM((NT, S, T), bf16), sems=pltpu.SemaphoreType.DMA((9,)))
    return [landing, tied, other]


def _kernel(x_hbm, wqkv_hbm, wo_hbm, w1_hbm, w2_hbm, c_hbm, wmod_hbm, o_hbm, raw, tied, mem):
    col = lambda t: slice(t * T, (t + 1) * T)
    k_s, v_s, out_s, sems = mem["k"], mem["v"], mem["out"], mem["sems"]

    x_in = lambda b: (x_hbm.at[b * BM:(b + 1) * BM], raw["x"][b].at[:BM])
    qkv_in = lambda p: (wqkv_hbm.at[:, p * D:(p + 1) * D], raw["wqkv"][p].at[:D])
    mod_in = lambda j: (wmod_hbm.at[:, j * D:(j + 1) * D], raw["wmod"][j].at[:D])
    waves = [[(c_hbm, raw["c"]), qkv_in(0)], [x_in(0)], [mod_in(1)], [mod_in(0)], [qkv_in(1)], [qkv_in(2)],
             [x_in(1)], [x_in(2), (wo_hbm, raw["wo"].at[:D]), mod_in(2), x_in(3)],
             [mod_in(3), mod_in(4), (w1_hbm, raw["w1"].at[:D]), mod_in(5), (w2_hbm, raw["w2"].at[:F])]]
    waves = [[pltpu.make_async_copy(src, dst, sems.at[i]) for src, dst in wave] for i, wave in enumerate(waves)]
    results = []

    def send(rows, t):
        results.append(pltpu.make_async_copy(out_s.at[t, rows], o_hbm.at[rows, col(t)], sems.at[0]))
        results[-1].start()

    now = dict(clock=0, passes=0, quiet=0, align=False, zero=None)
    starts = {}
    pending, ties, history, fresh, free, eager = [], {}, [], [], list(mem["tmp"]), []

    def rows_at(r0, n):
        if (r0, n) not in starts:
            starts[r0, n] = pl.multiple_of(now["zero"] + r0, min(n, 16))
        return pl.ds(starts[r0, n], n)

    def zero_rows(ref):
        n = 16 if ref.dtype == bf16 else 8
        return (0,) * (len(ref.shape) - 2), ref.shape[-2] - n, n

    def put(ref, idx, r0, v):
        if not now["passes"]:
            ref[idx + (slice(r0, r0 + v.shape[0]),)] = v.astype(ref.dtype)
            return
        ref[idx + (rows_at(r0, v.shape[0]),)] = v.astype(ref.dtype)
        if not any(ref is p for p in pending):
            pending.append(ref)

    def tie():
        words = []
        for ref in pending:
            idx, r0, _ = zero_rows(ref)
            if ref.dtype == bf16:
                words.append(ref.bitcast(u32)[idx + (slice(r0 // 2, r0 // 2 + 8),)])
            else:
                words.append(pltpu.bitcast(ref[idx + (slice(r0, r0 + 8),)], u32))
        pending.clear()
        while len(words) > 1:
            words.append(words.pop() | words.pop())
        return words[0]

    def hold(ref, lag):
        for t, m, r in reversed(history):
            if t <= now["clock"] - lag:
                v = pltpu.bitcast(m[r:r + 8], u32) if ref.dtype == u32 else m[r:r + 8].astype(ref.dtype)
                ref[zero_rows(ref)[0] + (rows_at(ref.shape[-2] - SPARE, 8), col(0))] = v
                return

    def keep(value, uses):
        cell = dict(value=value, uses=uses, ref=None)
        fresh.append(cell)

        def read():
            cell["uses"] -= 1
            if cell["ref"] is None:
                return value
            if cell["uses"] == 0:
                free.append(cell["ref"])
            return cell["ref"][:value.shape[0]]
        return read

    def mxu_pass(a_ref, w_ref, o, k, n, lo, rows, counts=True):
        unit = (now["passes"] - (not counts)) % 4
        if unit == 0:
            yield 0
            now["passes"] += 1
            for cell in fresh:
                if cell["uses"]:
                    cell["ref"] = free.pop(0)
                    cell["ref"][rows_at(0, cell["value"].shape[0])] = cell["value"]
            fresh.clear()
            ties.clear()
            for r in range(0, rows, 16):
                yield 16
                if pending and now["clock"] >= now["quiet"]:
                    ties[r] = (tie(), now["align"] or rows <= QB)
                    now["align"] = False
                now["clock"] += 16
        else:
            now["passes"] += counts
        a = a_ref.bitcast(u32)[o, k, lo // 2:(lo + rows) // 2]
        mine = {r // 2: z for r, (z, everyone) in ties.items() if counts and (everyone or unit == 3)}
        if mine:
            a = jnp.concatenate([a[r:r + 8] | mine[r] if r in mine else a[r:r + 8]
                                 for r in range(0, rows // 2, 8)], axis=0)
        w = w_ref.bitcast(u32)[o, n, k * T // 2:(k + 1) * T // 2]
        m = jnp.dot(pltpu.bitcast(a, bf16), pltpu.bitcast(w, bf16), preferred_element_type=f32)
        if unit == 0:
            history.extend((now["clock"] - rows + r, m, r) for r in range(0, rows, 16))
        return m

    def silu_c():
        c = raw["c"][...].astype(f32)
        sc = c * jax.nn.sigmoid(c)
        for t in range(NT):
            mem["sc"][col(t)] = jnp.broadcast_to(sc[:, col(t)], (T, T)).T
        n = pltpu.bitcast(jnp.broadcast_to(c[:, :T], (8, T)), jnp.int32) & 255
        now["zero"] = ((n * n + n) & 1)[0, 0]

    def gen_mod(j, mul=1.0, add=0.0):
        for r in range(NT):
            for t in range(NT):
                hold(raw["wmod"][j], NEAR)
                p = raw["wmod"][j][col(r), col(t)].astype(f32) * mem["sc"][col(r)]
                acc = _tree(jnp.add, [p[i:i + 8] for i in range(0, T, 8)])
                if r:
                    acc = acc + tied["mod"][j][t, :8]
                if r == NT - 1:
                    acc = jnp.broadcast_to(jnp.sum(acc, axis=0, keepdims=True) * mul + add, (8, T))
                put(tied["mod"][j], (t,), 0, acc)
                yield 50

    def mod(j, t, rows):
        return jnp.concatenate([tied["mod"][j][t, :8]] * (rows // 8), axis=0)

    def gen_rhs(src, lag, tile, dst, r):
        for k in range(2):
            for n in range(2):
                hold(src, lag)
                _operands(_RHS, lambda i, j: tile(2 * i + k, 2 * j + n), lambda o, v: put(dst, (o, n), k * T + r, v))
                yield 30

    def gen_wqkv(p):
        src = raw["wqkv"][p]
        lane = lax.broadcasted_iota(jnp.int32, (8, T), 1)
        pos = lane >> 3
        for half, buf in enumerate(tied["perm"]):
            for t in range(NT):
                u = (pos - t) & 3
                idx = (lane & 7) * DH + u * 4 + (((pos - u) & 15) >> 2)
                for r in range(0, T // 2, 16):
                    hold(src, FAR)
                    for k in range(NT):
                        r0 = k * T + half * T // 2 + r
                        w = pltpu.bitcast(src[r0:r0 + 16, col(t)], u32)
                        put(buf, (k * NT + t,), r // 2, jnp.take_along_axis(w, idx, axis=1))
                    yield 24
        slot = pos & 3
        for r in range(0, T, 16):
            buf, r2 = tied["perm"][r // (T // 2)], r % (T // 2) // 2

            def tile(k, u):
                g = [buf[k * NT + (i - u) % 4, r2:r2 + 8] for i in range(4)]
                y = jnp.where(slot < 2, jnp.where(slot == 0, g[0], g[1]), jnp.where(slot == 2, g[2], g[3]))
                y = pltpu.bitcast(pltpu.roll(y, T - 8 * u, 1) if u else y, bf16).astype(f32)
                return y if p else y * (DH ** -0.5 * LOG2E)
            yield from gen_rhs(buf, FAR, tile, tied["bq"][p], r)

    def gen_wo():
        for t in range(NT):
            for h0 in range(0, H, 8):
                hold(raw["wo"], NEAR)
                for h in range(h0, h0 + 8):
                    w = raw["wo"][h * DH:(h + 1) * DH, col(t)].astype(f32)
                    mem["wo32"][t, h * (DH + 1):h * (DH + 1) + DH] = w * mod(2, t, DH)
                yield 40
        for r in range(0, T, 16):
            def tile(k, t):
                d, h = divmod(k * T + r, H)
                return mem["wo32"][t, pl.ds(h * (DH + 1) + d, 16, stride=DH + 1), :]
            yield from gen_rhs(mem["wo32"], NEAR, tile, tied["bo"], r)

    def gen_w1():
        for g in range(FT // 2):
            for r in range(0, 2 * T, 16):
                hold(raw["w1"], NEAR)
                tile = lambda i, j: raw["w1"][2 * i * T + r:2 * i * T + r + 16, col(2 * g + j)].astype(f32)
                _operands(_RHS, tile, lambda o, v: put(tied["b1"], (o, g), r, v))
                yield 30

    def gen_w2():
        for r in range(0, T, 16):
            tile = lambda k, n: raw["w2"][k * T + r:k * T + r + 16, col(n)].astype(f32)
            for g in range(3):
                for outer in SHARE:
                    hold(raw["w2"], NEAR)
                    _operands2(_RHS, outer, lambda i, j: tile(4 * g + i, j),
                               lambda o, v: put(tied["b2"], (o, 0), g * T + r, v))
                    yield 24 + 17 * len(outer)
            for n in range(2):
                hold(raw["w2"], NEAR)
                _operands(_RHS, lambda i, j: tile(12 + i, 2 * j + n), lambda o, v: put(tied["b2r"], (o, n), r, v))
                yield 30

    def gen_lhs(src, tile, dst, r, ops):
        for k in range(2):
            hold(src, NEAR)
            _operands(_LHS, lambda i, j: tile(i, 2 * j + k), lambda o, v: put(dst, (o, k), r, v))
            yield ops

    part = lambda r0: r0 % QB // (QB // 2)

    def gen_stats(src, load, stats):
        order = sorted(range(0, BM, 16), key=part)
        for r0 in order:
            if r0 % 64 == 0:
                hold(src, FAR)
            total = jnp.sum(_tree(jnp.add, [load(r0, t) for t in range(NT)]), axis=-1, keepdims=True)
            put(stats[0][part(r0)], (), r0, jnp.broadcast_to(total * (1.0 / D), (16, T)))
            yield 20
        for r0 in order:
            hold(src, FAR)
            xc = [load(r0, t) - stats[0][part(r0)][r0:r0 + 16] for t in range(NT)]
            var = jnp.sum(_tree(jnp.add, [v * v for v in xc]), axis=-1, keepdims=True) * (1.0 / D)
            put(stats[1][part(r0)], (), r0, jnp.broadcast_to(lax.rsqrt(var + 1e-5), (16, T)))
            yield 46

    def scaled(load, stats, scale, r0, t):
        mean, rstd = (s[part(r0)][r0:r0 + 16] for s in stats)
        return (load(r0, t) - mean) * rstd * mod(scale, t, 16)

    ln1 = lambda b: (raw["x"][b], lambda r0, t: raw["x"][b][r0:r0 + 16, col(t)].astype(f32), tied["stats"][0])
    ln2 = lambda b: (mem["x1"][b], lambda r0, t: mem["x1"][b][t, r0:r0 + 16], tied["stats"][1])

    def gen_ln(which, dst, scale, shift):
        yield from gen_stats(*which)
        for r in range(0, HB, 16):
            tile = lambda i, t: scaled(*which[1:], scale, i * HB + r, t) + mod(shift, t, 16)
            yield from gen_lhs(which[0], tile, dst, r, 53)

    window = lambda r0, w: slice(HALO + r0 - DIL * w, HALO + r0 - DIL * w + 8)

    def att_logits(r0, logit):
        q_ref = mem["q"][r0 // BM]
        for w0 in (0, W // 2):
            hold(q_ref, FAR)
            q = [q_ref[t, r0 % BM:r0 % BM + 8] for t in range(NT)]
            for w in range(w0, w0 + W // 2):
                p = _tree(jnp.add, [q[t] * k_s[t, window(r0, w)] for t in range(NT)])
                put(logit, (w,), 0, p + pltpu.roll(p, 64, 1))
            yield 32

    def att_probs(r0, logit, prob):
        hold(logit, FAR)
        lg = [logit[w, :8] for w in range(W)]
        lg = [p + pltpu.roll(p, 32, 1) for p in lg]
        for w in range(W):
            if r0 < DIL * w:
                row = lax.broadcasted_iota(jnp.int32, (8, T), 0)
                lg[w] = jnp.where(row >= DIL * w - r0, lg[w], -1e9 * LOG2E)
        top = _tree(jnp.maximum, lg)
        for w in range(W):
            put(prob, (w,), 0, jnp.exp2(lg[w] - top))
        yield 32

    def att_values(r0, prob, att, o0):
        for t0 in (0, NT // 2):
            hold(prob, NEAR)
            e = [prob[w, :8] for w in range(W)]
            if t0 == 0:
                den = _tree(jnp.add, e)
                inv = pltpu.reciprocal(den, approx=True)
                inv = inv * (2.0 - den * inv)
            for t in range(t0, t0 + NT // 2):
                put(att, (t,), o0, _tree(jnp.add, [e[w] * v_s[t, window(r0, w)] for w in range(W)]) * inv)
            yield 38

    def gen_att(b):
        if b == 0:
            for t in range(NT):
                k_s[t, :HALO] = jnp.zeros((HALO, T), f32)
                v_s[t, :HALO] = jnp.broadcast_to(v_s[t, HALO:HALO + 1], (HALO, T))
        units = [(r, i, z) for r in range(0, HB, 16) for i in range(2) for z in (0, 8)]
        row = lambda u: b * BM + units[u][1] * HB + units[u][0] + units[u][2]
        logit, prob = (lambda u: tied["logit"][u % 8]), (lambda u: tied["prob"][u % 8])
        for u in range(len(units) + 5):
            steps = {}
            if u < len(units):
                steps["l"] = att_logits(row(u), logit(u))
            if 0 <= u - 3 < len(units):
                steps["p"] = att_probs(row(u - 3), logit(u - 3), prob(u - 3))
            if u >= 5:
                r, i, z = units[u - 5]
                att = tied["att"][r // 16 % 4]
                steps["v"] = att_values(row(u - 5), prob(u - 5), att, i * 16 + z)
            for kind in "vlvpl":
                if kind in steps:
                    yield next(steps[kind])
            if u >= 5 and (i, z) == (1, 8):
                yield from gen_lhs(att, lambda i, t: att[t, i * 16:i * 16 + 16], tied["ao"][b % 2], r, 17)

    def gen_hidden(b, g):
        hid = mem["hid"][b % 2]
        for r in range(0, QB if g < 3 else HB, 16):
            if g == 3:
                _operands(_LHS, lambda i, j: hid[12 + j][i * HB + r:i * HB + r + 16],
                          lambda o, v: put(tied["a2r"][b % 2], (o, 0), r, v))
                yield 24
                continue
            for outer in SHARE:
                _operands2(_LHS, outer, lambda i, j: hid[4 * g + j][i * QB + r:i * QB + r + 16],
                           lambda o, v: put(tied["a2"][b % 2], (o, g), r, v))
                yield 10 + 17 * len(outer)

    def matmul(a_ref, w_ref, n, done, last=False):
        step = _combiner(keep)
        for o in range(7):
            pieces = []
            for lo, rows in ((0, QB), (QB, QB)) if last and o == 6 else ((0, HB),):
                m = yield from mxu_pass(a_ref, w_ref, o, 0, n, lo, rows)
                pieces.append(m + (yield from mxu_pass(a_ref, w_ref, o, 1, n, lo, rows)))
            block = step(o, jnp.concatenate(pieces, axis=0))
            if block:
                done(*block)

    def gen_qkv(b, p):
        dst, r0 = ((mem["q"][b], 0), (k_s, HALO + b * BM), (v_s, HALO + b * BM))[p]
        for n in range(2):
            def done(i, j, m):
                dst[2 * j + n, r0 + i * HB:r0 + (i + 1) * HB] = m
            yield from matmul(tied["aq"][b % 2], tied["bq"][p], n, done)

    def gen_proj(b):
        for n in range(2):
            def done(i, j, m):
                rows = slice(i * HB, (i + 1) * HB)
                mem["x1"][b][2 * j + n, rows] = raw["x"][b][rows, col(2 * j + n)].astype(f32) + m
            yield from matmul(tied["ao"][b % 2], tied["bo"], n, done)

    def gen_up(b):
        def paced(g):
            yield 200, 0
            for ops in gen_hidden(b, g):
                yield (1.33 * ops if g < 3 else 56), ops

        for g in range(FT // 2):
            def done(i, j, m):
                mem["hid"][b % 2][2 * g + j][rows_at(i * HB, HB)] = m + m * jnp.tanh(m)
            yield from matmul(tied["a1"][b % 2], tied["b1"], g, done, g == FT // 2 - 1)
            if b == 0 and (g % 2 or g == FT // 2 - 1):
                eager.append(paced(g // 2))

    def gen_down(b):
        while eager:
            list(eager.pop(0))
        a2, a2r = tied["a2"][b % 2], tied["a2r"][b % 2]
        outer = [[_combiner(keep) for _ in range(2)] for _ in range(2)]
        for o in range(7):
            inner = _combiner(keep)
            for p in range(7):
                m = keep((yield from mxu_pass(a2, tied["b2"], 7 * o + p, 0, 0, 0, QB)), 1)
                if (o, p) == (6, 6):
                    pieces, cut = [], 3 * QB // 4
                    for lo, rows in ((0, cut), (cut, QB - cut)):
                        d = yield from mxu_pass(a2, tied["b2"], 48, 1, 0, lo, rows)
                        d = d + (yield from mxu_pass(a2, tied["b2"], 48, 2, 0, lo, rows, not lo))
                        pieces.append(d + (yield from mxu_pass(a2r, tied["b2r"], 6, 0, 1, QB + lo, rows, not lo)))
                    block = inner(p, m() + jnp.concatenate(pieces, axis=0))
                else:
                    rest = [(a2, tied["b2"], 7 * o + p, k, 0, 0, QB) for k in (1, 2)]
                    if p > 4:
                        rest.append((a2r, tied["b2r"], o, 0, p - 5, (p - 5) * QB, QB))
                    for args in rest:
                        d = yield from mxu_pass(*args)
                        m = keep(m() + d, 1)
                    block = inner(p, m())
                    if block and p < 5:
                        m = keep(block[2], 1)
                        d = yield from mxu_pass(a2r, tied["b2r"], o, 0, block[1], block[0] * QB, QB)
                        block = block[:2] + (m() + d,)
                final = block and outer[block[0]][block[1]](o, block[2])
                if final:
                    r0, t = final[0] * HB + block[0] * QB, 2 * final[1] + block[1]
                    rows = slice(b * BM + r0, b * BM + r0 + QB)
                    out_s[t, rows] = (mem["x1"][b][t, r0:r0 + QB] + mod(5, t, QB) * final[2]).astype(bf16)
                    if b == NB - 1:
                        send(rows, t)
        if b < NB - 1:
            for t in range(NT):
                send(slice(b * BM, (b + 1) * BM), t)

    def after(wave, gen):
        if wave is not None:
            for copy in waves[wave]:
                copy.wait()
            now["quiet"] = now["clock"] + (2000 if wave < 6 else FAR)
            history.clear()
            pending.clear()
        now["align"] = True
        yield from gen

    def head(gen, rounds):
        for c in gen:
            rounds -= c == 0
            if rounds < 0:
                return
            yield c

    for wave in waves:
        for copy in wave:
            copy.start()
    for ref in jax.tree.leaves(tied):
        idx, r0, n = zero_rows(ref)
        ref[idx + (slice(r0, r0 + n),)] = jnp.zeros((n, T), ref.dtype)
    list(after(0, gen_wqkv(0)))
    silu_c()
    list(after(1, gen_stats(*ln1(0))))
    list(after(2, gen_mod(1, add=1.0)))
    early = {(r0, t): scaled(*ln1(0)[1:], 1, r0, t) for r0 in range(0, BM, 16) for t in range(NT)}
    list(after(3, gen_mod(0)))
    for r in range(0, HB, 16):
        list(gen_lhs(None, lambda i, t: early[i * HB + r, t] + mod(0, t, 16), tied["aq"][0], r, 0))

    pool = {}
    for b in range(NB):
        pool.update({"Q%d%d" % (b, p): (7 * HB, gen_qkv(b, p)) for p in range(3)})
        pool.update({"O%d" % b: (7 * HB, gen_proj(b)), "F%d" % b: (49 * HB // 2, gen_up(b)),
                     "G%d" % b: (175 * QB // 4, gen_down(b))})
    stages = []
    for item in ORDER.split(","):
        name, _, rounds = item.partition(":")
        cycles, gen = pool.pop(name)
        if rounds:
            first = int(rounds) * (QB if name[0] == "G" else HB)
            pool[name + "b"] = (cycles - first, gen)
            cycles, gen = first, head(gen, int(rounds))
        stages.append((name, cycles, LOAD.get(name, LOAD[name[0]]), after(ARRIVALS.get(name), gen)))
    assert not pool
    names = [st[0] for st in stages]
    assert all(names.index("F%d" % (b + 2)) > max(i for i, n in enumerate(names) if n.startswith("G%d" % b))
               for b in range(NB - 2))
    chain = lambda *gens: (ops for gen in gens for ops in gen)
    shared = lambda base: sum(base + 17 * len(outer) for outer in SHARE)
    dense = [(1728, "Q00", "Q01", gen_wqkv(1)), (1728, "Q00b", "Q02", gen_wqkv(2)),
             (2400, "Q10", "O0", chain(gen_mod(2), gen_wo())), (3360, "O0", "F0", gen_w1()),
             (480 + 24 * shared(24), "O0", "G0", gen_w2())]
    tasks = [(800, "O0", "G0", gen_mod(5))]
    for b in range(NB):
        norm = gen_ln(ln2(b), tied["a1"][b % 2], 4, 3)
        if b:
            tasks.append((3808, ("Q01", "Q10", "Q12")[b - 1], "Q%d0" % b, gen_ln(ln1(b), tied["aq"][b % 2], 1, 0)))
            tasks.append((3808, "O%d+" % b, "F%d" % b, norm))
            dense.append((384 + 24 * shared(10), "F%d" % b, "G%d" % b, chain(*[gen_hidden(b, g) for g in range(4)])))
        else:
            tasks.append((5408, "O0", "F0", chain(gen_mod(4, 0.5, 0.5), gen_mod(3, 0.5), norm)))
        tasks.append((11552, ("Q02+", "Q12+", "O0", "O1")[b], "O%d" % b, gen_att(b)))
    _emit(stages, (tasks, dense), eager)
    for copy in results:
        copy.wait()


@jax.jit
def pallas_adaLN_cond__sliding_local_dilated__dense_activation_silu__prompt_kernel(
        A_x, A_wqkv, A_wo, B_x, B_w1, B_w2, c, w_mod):
    del B_x
    out = pl.pallas_call(
        _kernel,
        in_specs=[pl.BlockSpec(memory_space=pl.ANY)] * 7,
        out_specs=pl.BlockSpec(memory_space=pl.ANY),
        out_shape=jax.ShapeDtypeStruct((S, D), A_x.dtype),
        scratch_shapes=_scratch(),
        compiler_params=pltpu.CompilerParams(vmem_limit_bytes=100 * 1024 * 1024),
        name="adaln_block",
    )(A_x.reshape(S, D), A_wqkv, A_wo, B_w1, B_w2, c, w_mod)
    return out.reshape(A_x.shape)
```
